```python
import jax
import jax.numpy as jnp

def _softmax(x, axis=-1):
    return jax.nn.softmax(x, axis=axis)
def _gelu(x):
    return jax.nn.gelu(x, approximate=True)
def _silu(x):
    return jax.nn.silu(x)
def _sigmoid(x):
    return jax.nn.sigmoid(x)
def _layernorm(x, axis=-1, eps=1e-5):
    m = jnp.mean(x, axis=axis, keepdims=True)
    v = jnp.var(x, axis=axis, keepdims=True)
    return (x - m) / jnp.sqrt(v + eps)
def _scatter_add(tgt, idx, src, axis=0):
    return tgt.at[idx].add(src)
def _segment_sum(src, seg, n):
    return jax.ops.segment_sum(src, seg, n)
class _Rng:
    def __init__(self, key):
        self._k = key
    def _next(self):
        self._k, sub = jax.random.split(self._k)
        return sub
    def normal(self, shape):
        return jax.random.normal(self._next(), shape, dtype=jnp.bfloat16)
    def randint(self, lo, hi, shape):
        return jax.random.randint(self._next(), shape, lo, hi, dtype=jnp.int32)
    def uniform(self, shape, lo=0.0, hi=1.0):
        return jax.random.uniform(self._next(), shape, jnp.bfloat16, lo, hi)
    def permutation(self, n):
        return jax.random.permutation(self._next(), n)


kernel_name = 'gated_mix__sliding_local_dilated__swiglu_ffn__prompt'

def _fwd_setup_inputs():
    _rng = _Rng(jax.random.key(int.from_bytes(__import__("os").urandom(4), "little")))
    _w = (lambda a: (lambda t: t.astype(jnp.bfloat16) if jnp.issubdtype(t.dtype, jnp.floating) else t)(jnp.asarray(a)))
    def _A_setup():
        B, S, D = 1, 2048, 448
        return {
            "x": _w((lambda *s: _rng.normal(s) * 0.05)(B, S, D)),
            "wqkv": _w((lambda *s: _rng.normal(s) * 0.05)(D, 3 * D)),
            "wo": _w((lambda *s: _rng.normal(s) * 0.05)(D, D)),
        }
    _A_in = _A_setup()

    def _B_setup():
        B, S, D, F = 1, 2048, 448, 1792
        return {
            "x": _w((lambda *s: _rng.normal(s) * 0.05)(B, S, D)),
            "w_gate": _w((lambda *s: _rng.normal(s) * 0.05)(D, F)),
            "w_up": _w((lambda *s: _rng.normal(s) * 0.05)(D, F)),
            "w_down": _w((lambda *s: _rng.normal(s) * 0.05)(F, D)),
        }
    _B_in = _B_setup()

    return {
        "A_x": _A_in["x"],
        "A_wqkv": _A_in["wqkv"],
        "A_wo": _A_in["wo"],
        "B_x": _B_in["x"],
        "B_w_gate": _B_in["w_gate"],
        "B_w_up": _B_in["w_up"],
        "B_w_down": _B_in["w_down"],
        "gate_w": _w((lambda *s: _rng.normal(s) * 0.05)(448)),
    }

def _fwd_reference(A_x, A_wqkv, A_wo, B_x, B_w_gate, B_w_up, B_w_down, gate_w):
    def _A_ref(x, wqkv, wo):
        B, S, D = x.shape
        H = 16; Dh = D // H
        W, dil = 8, 2
        qkv = (lambda x, *d: x.transpose(*d))((x @ wqkv).reshape(B, S, 3, H, Dh), 2, 0, 3, 1, 4)
        q, k, v = qkv[0], qkv[1], qkv[2]
        scale = Dh ** -0.5
        pos = jnp.arange(S)
        off = jnp.arange(W) * dil
        idx = pos[:, None] - off[None, :]
        mask = idx >= 0
        idx_c = jnp.where(mask, idx, 0).reshape(-1)
        kg = k[:, :, idx_c, :].reshape(B, H, S, W, Dh)
        vg = v[:, :, idx_c, :].reshape(B, H, S, W, Dh)
        logits = jnp.einsum("bhsd,bhswd->bhsw", q, kg) * scale
        logits = jnp.where(mask[None, None, :, :], logits, -1e9)
        attn = _softmax(logits, axis=-1)
        o = jnp.einsum("bhsw,bhswd->bhsd", attn, vg)
        return (lambda x, *d: x.transpose(*d))(o, 0, 2, 1, 3).reshape(B, S, D) @ wo

    def _B_ref(x, w_gate, w_up, w_down):
        g = _silu(x @ w_gate)
        u = x @ w_up
        return (g * u) @ w_down

    x = A_x
    g = _sigmoid((x * gate_w).sum(-1, keepdims=True))
    a = _A_ref(x, A_wqkv, A_wo)
    b = _B_ref(x, B_w_gate, B_w_up, B_w_down)
    return g * a + (1 - g) * b


def setup_inputs():
    _inp = _fwd_setup_inputs()
    _gk = jax.random.fold_in(jax.random.key(int.from_bytes(__import__("os").urandom(4), "little")), 2**31 - 1)
    _shapes = [[1, 2048, 448]]
    _dtypes = ['bfloat16']
    _gks = jax.random.split(_gk, len(_shapes))
    _gs = [jax.random.normal(k, s, dtype=jnp.dtype(d)) * 0.05 for k, s, d in zip(_gks, _shapes, _dtypes)]
    _inp["grad_out"] = _gs[0]
    return _inp

def reference(A_x, A_wqkv, A_wo, B_w_gate, B_w_up, B_w_down, gate_w, B_x, grad_out):
    _const = dict(B_x=B_x)
    def _f(*_d):
        return _fwd_reference(**{'A_x': _d[0], 'A_wqkv': _d[1], 'A_wo': _d[2], 'B_w_gate': _d[3], 'B_w_up': _d[4], 'B_w_down': _d[5], 'gate_w': _d[6], **_const})
    _out, _vjp = jax.vjp(_f, A_x, A_wqkv, A_wo, B_w_gate, B_w_up, B_w_down, gate_w)
    _grads = _vjp(grad_out)
    _out0 = jnp.asarray(_out)
    return (_out0, *[jnp.asarray(_g) for _g in _grads])
```

```python
import functools
import jax
import jax.numpy as jnp
import jax.experimental.pallas as pl
import jax.experimental.pallas.tpu as pltpu

bf = jnp.bfloat16
f32 = jnp.float32
S, D, F, H, DH, W = 2048, 448, 1792, 16, 28, 8
NQ = 1408
NO = 512
TS = 256
WR = TS + 32
WS = TS + 40
RG = 8
TFF = 256
CG = 1024
TFB = 128
NFF = F // TFF
NFB = F // TFB
NT_ = S // TS
SP = S + 32
QKV, DO, PB, OB = 0, 11, 15, 31
NB = 46
SCALE = DH ** -0.5
CEXP = SCALE * 1.4426950408889634
NEG = -1e30

NN = (((1,), (0,)), ((), ()))
NT = (((1,), (1,)), ((), ()))
TN = (((0,), (0,)), ((), ()))


def dot(a, b, dn):
    return jax.lax.dot_general(a, b, dn, preferred_element_type=f32)


def U(x):
    return pltpu.bitcast(x, bf)


def Pk(x):
    return pltpu.bitcast(x, f32)


def sigmoid(x):
    return 0.5 * jnp.tanh(0.5 * x) + 0.5


def prow(t, d):
    if d < 24:
        return 384 * t + 16 * d
    return (1344, 1216, 1152)[t] + 16 * (d - 24)


def sum_(xs):
    return functools.reduce(lambda a, b: a + b, xs)


def masks():
    g = jax.lax.broadcasted_iota(jnp.int32, (RG, 128), 1) // 16
    m1 = [((g + s) % 8) < 4 for s in range(4)]
    m2 = [((g + s) % 4) >= 2 for s in range(2)]
    m3 = (g % 2) == 1
    return m1, m2, m3


def comb(m, a, b, sh):
    return jnp.where(m, a, b) + pltpu.roll(jnp.where(m, b, a), sh, 1)


def split(m, z, sh):
    r = pltpu.roll(z, 128 - sh, 1)
    return jnp.where(m, z, r), jnp.where(m, r, z)


def expand8(z, ms):
    m1, m2, m3 = ms
    va, vb = split(m3, z, 16)
    ua, ub = split(m2[0], va, 32)
    ua2, ub2 = split(m2[1], vb, 32)
    x0, x1 = split(m1[0], ua, 64)
    x2, x3 = split(m1[2], ub, 64)
    x4, x5 = split(m1[1], ua2, 64)
    x6, x7 = split(m1[3], ub2, 64)
    return [x0, x1, x2, x3, x4, x5, x6, x7]


def allred(t):
    t = t + pltpu.roll(t, 64, 1)
    t = t + pltpu.roll(t, 32, 1)
    return t + pltpu.roll(t, 16, 1)


def softmax_fb(L, A):
    m = functools.reduce(jnp.maximum, L)
    E = [jnp.exp2((l - m) * CEXP) for l in L]
    r = 1.0 / sum_(E)
    P = [e * r for e in E]
    sm = sum_([p * a for p, a in zip(P, A)])
    return P, [(p * SCALE) * (a - sm) for p, a in zip(P, A)]


class Att:
    def __init__(self, at, z):
        self.at, self.z = at, pl.multiple_of(z, 256)

    def ld(self, b, s):
        return self.at[b, s:s + RG, :]

    def st(self, b, s, v, n=RG):
        self.at[b, pl.ds(self.z + s, n), :] = v

    def ldz(self, b, s):
        return self.at[b, pl.ds(self.z + s, RG), :]

    def sts(self, b, s, v):
        self.at[b, s:s + RG, :] = v

    def tu(self, g):
        ld, ldz = self.ld, self.ldz
        q = [ldz(0, g), ld(1, g), ld(2, g), ld(10, g)]
        dd = [ldz(DO, g)] + [ld(DO + b, g) for b in range(1, 4)]
        T, Uu = [], []
        for w in range(W):
            s = g - 2 * w
            a9 = ld(9, s)
            T.append(q[0] * ld(3, s) + q[1] * ld(4, s) + q[2] * ld(5, s) + q[3] * a9)
            Uu.append(dd[0] * ld(6, s) + dd[1] * ld(7, s) + dd[2] * ld(8, s) + dd[3] * a9)
        return T + Uu

    def phase1_first_rows(self):
        for g in (16, 24):
            tu = [allred(x) for x in self.tu(g)]
            row = jax.lax.broadcasted_iota(jnp.int32, (RG, 128), 0) + (g - 16)
            L = [jnp.where(row >= 2 * w, tu[w], NEG) for w in range(W)]
            P, DL = softmax_fb(L, tu[W:])
            for w in range(W):
                self.st(PB + w, g, P[w])
                self.st(PB + 8 + w, g, DL[w])

    def phase1(self, G, ms):
        m1, m2, m3 = ms

        def lvl1(y, m):
            a = self.tu(G + 8 * y)
            b = self.tu(G + 8 * y + 8)
            r = [comb(m, p, q_, 64) for p, q_ in zip(a, b)]
            for k in range(16):
                self.sts(PB + k, G + 8 * y, r[k])

        lvl1(0, m1[0]); lvl1(2, m1[2]); lvl1(4, m1[1]); lvl1(6, m1[3])
        zz = []
        for k in range(16):
            va = comb(m2[0], self.ld(PB + k, G), self.ld(PB + k, G + 16), 32)
            vb = comb(m2[1], self.ld(PB + k, G + 32), self.ld(PB + k, G + 48), 32)
            zz.append(comb(m3, va, vb, 16))
        P, DL = softmax_fb(zz[:8], zz[8:])
        for w in range(W):
            xp = expand8(P[w], ms)
            xd = expand8(DL[w], ms)
            for y in range(8):
                self.sts(PB + w, G + 8 * y, xp[y])
                self.sts(PB + 8 + w, G + 8 * y, xd[y])

    def phase2(self, g16, part):
        ld = self.ld

        def rows(g):
            def acc(coef, b, sgn):
                return sum_([coef[w] * ld(b, g + sgn * 2 * w) for w in range(W)])
            if part == 'o':
                P = [(self.ldz if g16 == 16 else ld)(PB + w, g) for w in range(W)]
                return {k: acc(P, b, -1) for k, b in enumerate((6, 7, 8, 9))}
            if part == 'q':
                DL = [ld(PB + 8 + w, g) for w in range(W)]
                return {k: acc(DL, b, -1) for k, b in zip((4, 5, 6, 14), (3, 4, 5, 9))}
            Pf = [ld(PB + w, g + 2 * w) for w in range(W)]
            if part == 'k':
                DLf = [ld(PB + 8 + w, g + 2 * w) for w in range(W)]
                res = {7 + b: acc(DLf, b, +1) for b in range(3)}
                res[13] = acc(DLf, 10, +1) + acc(Pf, DO + 3, +1)
                return res
            return {10 + b: acc(Pf, DO + b, +1) for b in range(3)}

        a = rows(g16)
        self.st(OB, WR - RG, a[max(a)])
        b = rows(g16 + 8)
        for k in sorted(a):
            pk = jnp.concatenate([a[k], b[k]], axis=0).astype(bf)
            self.st(OB + k, (g16 - 16) // 2, Pk(pk))

    def tile(self):
        ms = masks()
        for j in range(4):
            self.phase1(32 + 64 * j, ms)
        for g16 in range(16, 16 + TS, 16):
            for part in 'oqkv':
                self.phase2(g16, part)


def kernel(xat_h, wqkv_h, wo_h, wg_h, wu_h, wdt_h, gw_h, dyt_h,
           out_h, dx_h, dwqkv_h, dwo_h, dwg_h, dwu_h, dwdt_h, dgw_h,
           xat, dyt, wqkv, wo, wg, wu, wdt, gw,
           xat_p, dat_p, dbt_p, xar_p, dar_p, wg_p, wu_p, wT_p,
           wp_p, wpt_p, wop_p, wopt_p, hs_p, dgs_p, dus_p,
           bt, grow, gwcol, dwp, dwot, dgacc, at, nwin, perm,
           out_s, dx_s, dwqkv_s, dwo_s, dwg_s, dwu_s, dwdt_s, dgw_s,
           zs, isem, osem, fsem):
    cp = pltpu.make_async_copy

    def wcopies(j):
        sl = pl.ds(pl.multiple_of(j * TFF, TFF), TFF)
        return [cp(h.at[:, sl], v.at[:, sl], isem.at[9 + 3 * j + k])
                for k, (h, v) in enumerate(((wg_h, wg), (wu_h, wu), (wdt_h, wdt)))]

    xa_cols = (slice(0, 512), slice(512, 1024), slice(1024, 2048))
    c_xa = [cp(xat_h.at[:, c], xat.at[:, c], isem.at[k]) for k, c in zip((0, 1, 30), xa_cols)]
    c_gw, c_dyt, c_wqkv, c_wo = [cp(h, v, isem.at[2 + k]) for k, (h, v) in enumerate(
        ((gw_h, gw), (dyt_h, dyt), (wqkv_h, wqkv), (wo_h, wo)))]
    w0 = wcopies(0)
    for c in [c_gw, w0[0], c_xa[0], w0[1], c_xa[1], c_xa[2], c_dyt, w0[2]]:
        c.start()
    for j in range(1, NFF):
        for c in wcopies(j):
            c.start()
    c_wqkv.start()
    c_wo.start()

    zs[0] = 0
    dwp[...] = jnp.zeros_like(dwp)
    dwot[...] = jnp.zeros_like(dwot)
    dgacc[...] = jnp.zeros_like(dgacc)

    def act_ew(sh, cs, G, Uv, dh, wdc, first):
        sig = sigmoid(G)
        si = G * sig
        h = (si * Uv).astype(bf)
        hs_p[sh, cs] = Pk(h)
        dus_p[sh, cs] = Pk((dh * si).astype(bf))
        dgs_p[sh, cs] = Pk((dh * Uv * (sig + si * (1.0 - sig))).astype(bf))
        if first:
            bt[:, cs] = dot(wdc, h, NN)
        else:
            bt[:, cs] += dot(wdc, h, NN)

    def prefetch_wT(j):
        sl = pl.ds(pl.multiple_of(j * TFF, TFF), TFF)
        wgc, wuc = wg[:, sl], wu[:, sl]
        wg_p[:, sl] = Pk(wgc)
        wu_p[:, sl] = Pk(wuc)
        wT_p[0] = Pk(wgc.T)
        wT_p[1] = Pk(wuc.T)
        wT_p[2] = Pk(wdt[:, sl].T)

    c_gw.wait()
    w0[0].wait()
    c_xa[0].wait()
    w0[1].wait()
    gwb = gw[...].reshape(1, D)
    row0 = jax.lax.broadcasted_iota(jnp.int32, (16, D), 0) == 0
    gw16 = jnp.where(row0, jnp.broadcast_to(gwb.astype(f32), (16, D)), 0.0).astype(bf)
    wgc, wuc = wg[:, 0:TFF], wu[:, 0:TFF]
    wg_p[:, 0:TFF] = Pk(wgc)
    wu_p[:, 0:TFF] = Pk(wuc)
    wgTe = jnp.concatenate([wgc.T, gw16], axis=0)
    wuT = wuc.T

    def gate_cols(cs):
        xat_p[:, cs] = Pk(xat[:, cs])
        Ge = dot(wgTe, U(xat_p[:, cs]), NN)
        grow[:, cs] = sigmoid(Ge[TFF:TFF + 1, :])
        return Ge[0:TFF]

    def up_cols(cs):
        return dot(wuT, U(xat_p[:, cs]), NN)

    qa, qb, qc, qd = [slice(512 * k, 512 * (k + 1)) for k in range(4)]
    Ga = gate_cols(qa)
    Ua = up_cols(qa)
    gwcol[...] = jnp.broadcast_to(gwb.astype(f32), (128, D)).T
    c_xa[1].wait()
    Gb = gate_cols(qb)
    Ub = up_cols(qb)
    c_xa[2].wait()
    Gcd = gate_cols(slice(1024, 2048))
    Uc = up_cols(qc)
    c_dyt.wait()
    w0[2].wait()
    for c in wcopies(1):
        c.wait()
    Ud = up_cols(qd)
    for c in range(S // 128):
        sl = slice(128 * c, 128 * (c + 1))
        g = grow[:, sl]
        dy = dyt[:, sl].astype(f32)
        dat_p[:, sl] = Pk((g * dy).astype(bf))
        dbt_p[:, sl] = Pk(((1.0 - g) * dy).astype(bf))
    wdc = wdt[:, 0:TFF]
    wdT = wdc.T
    cg0, cg1 = slice(0, CG), slice(CG, S)
    dh0 = dot(wdT, U(dbt_p[:, cg0]), NN)
    dh1 = dot(wdT, U(dbt_p[:, cg1]), NN)
    sh0 = slice(0, TFF // 2)
    act_ew(sh0, cg0, jnp.concatenate([Ga, Gb], axis=1), jnp.concatenate([Ua, Ub], axis=1), dh0, wdc, True)
    act_ew(sh0, cg1, Gcd, jnp.concatenate([Uc, Ud], axis=1), dh1, wdc, True)
    prefetch_wT(1)
    for j in range(2, NFF):
        for c in wcopies(j):
            c.wait()

    def ffn_act(j, carry):
        sl = pl.ds(pl.multiple_of(j * TFF, TFF), TFF)
        sh = pl.ds(pl.multiple_of(j * (TFF // 2), TFF // 2), TFF // 2)
        wdc = wdt[:, sl]

        def mm(c):
            cs = slice(c * CG, (c + 1) * CG)
            x = U(xat_p[:, cs])
            return dot(U(wT_p[0]), x, NN), dot(U(wT_p[1]), x, NN), dot(U(wT_p[2]), U(dbt_p[:, cs]), NN)

        n = S // CG
        nxt = mm(0)
        for c in range(n):
            cur = nxt
            if c + 1 < n:
                nxt = mm(c + 1)
            act_ew(sh, slice(c * CG, (c + 1) * CG), *cur, wdc, False)
        prefetch_wT(jnp.minimum(j + 1, NFF - 1))
        return carry

    jax.lax.fori_loop(1, NFF, ffn_act, 0)

    def ocopies(j):
        sl = pl.ds(pl.multiple_of(j * TFB, TFB), TFB)
        return [cp(v.at[:, sl], h.at[:, sl], fsem.at[k, j])
                for k, (v, h) in enumerate(((dwdt_s, dwdt_h), (dwg_s, dwg_h), (dwu_s, dwu_h)))]

    def wunit_parts(j):
        sl = pl.ds(pl.multiple_of(j * TFB, TFB), TFB)
        sh = pl.ds(pl.multiple_of(j * (TFB // 2), TFB // 2), TFB // 2)

        def p_d():
            dwdt_s[:, sl] = dot(U(dbt_p[...]), U(hs_p[sh, :]), NT).astype(bf)

        def p_g():
            dwg_s[:, sl] = dot(U(xat_p[...]), U(dgs_p[sh, :]), NT).astype(bf)

        def p_u():
            dwu_s[:, sl] = dot(U(xat_p[...]), U(dus_p[sh, :]), NT).astype(bf)
        return p_d, p_g, p_u

    c_wqkv.wait()
    c_wo.wait()
    for p in wunit_parts(NT_):
        p()
    for c in range(S // 128):
        sl = slice(128 * c, 128 * (c + 1))
        xar_p[64 * c:64 * (c + 1), :] = Pk(U(xat_p[:, sl]).T)
        dar_p[64 * c:64 * (c + 1), :] = Pk(U(dat_p[:, sl]).T)
    xar_p[S // 2:SP // 2, :] = jnp.zeros(((SP - S) // 2, D), f32)
    dar_p[S // 2:SP // 2, :] = jnp.zeros(((SP - S) // 2, D), f32)

    def lane_blocks_store(val, rows):
        for b in range(3):
            perm[b, 0:rows, :] = val[:, 128 * b:128 * (b + 1)]
        perm[3, 0:rows, :] = jnp.concatenate([val[:, 384:448], jnp.zeros((rows, 64), f32)], axis=1)

    def lane_blocks_gather(start, stride):
        parts = [perm[b, pl.ds(start, 16, stride=stride), :] for b in range(4)]
        return jnp.concatenate([parts[0], parts[1], parts[2], parts[3][:, 0:64]], axis=1)

    lane_blocks_store(wqkv[...].T.astype(f32), 3 * D)
    for t in range(3):
        for d in range(DH):
            r = prow(t, d) // 2
            wpt_p[r:r + 8, :] = Pk(lane_blocks_gather(D * t + d, DH).astype(bf))
    wpt_p[640:672, :] = jnp.zeros((32, D), f32)
    wp_p[...] = Pk(U(wpt_p[...]).T)
    lane_blocks_store(wo[...].astype(f32), D)
    for d in range(DH):
        wop_p[8 * d:8 * d + 8, :] = Pk(lane_blocks_gather(d, DH).astype(bf))
    wop_p[D // 2:NO // 2, :] = jnp.zeros(((NO - D) // 2, D), f32)
    wopt_p[...] = Pk(U(wop_p[...]).T)

    qkv0 = dot(U(xar_p[0:136, :]), U(wp_p[...]), NN)
    do0 = dot(U(dar_p[0:136, :]), U(wop_p[...]), NT)
    for b in range(15):
        v = qkv0[:, 128 * b:128 * (b + 1)] if b < 11 else do0[:, 128 * (b - 11):128 * (b - 10)]
        at[b, 0:16, :] = jnp.zeros((16, 128), f32)
        at[b, 16:288, :] = v
    for p in wunit_parts(NT_ + 1):
        p()
    Att(at, zs[0]).phase1_first_rows()

    def shuffle():
        for b in range(15):
            at[b, 0:32, :] = at[b, 256:288, :]
            at[b, 32:288, :] = nwin[b]
        for k in range(16):
            at[PB + k, 16:32, :] = at[PB + k, 272:288, :]

    for j in (NT_, NT_ + 1):
        for c in ocopies(j):
            c.start()

    def tcopies(i):
        sl = pl.ds(pl.multiple_of(i * TS, TS), TS)
        return [cp(out_s.at[:, sl], out_h.at[:, sl], osem.at[0, i]),
                cp(dx_s.at[:, sl], dx_h.at[:, sl], osem.at[1, i])]

    def tile_body(i, last):
        r0 = pl.multiple_of(i * TS, TS)
        tl = pl.ds(r0, TS)
        Att(at, zs[0]).tile()
        if not last:
            nx = pl.ds(pl.multiple_of((r0 + TS + 16) // 2, 8), TS // 2)
            qkv = dot(U(xar_p[nx, :]), U(wp_p[...]), NN)
            for b in range(11):
                nwin[b] = qkv[:, 128 * b:128 * (b + 1)]
            dd = dot(U(dar_p[nx, :]), U(wop_p[...]), NT)
            for b in range(4):
                nwin[11 + b] = dd[:, 128 * b:128 * (b + 1)]
        else:
            for p in wunit_parts(NT_ + 2):
                p()
        for p in wunit_parts(i):
            p()
        dxf = dot(U(wg_p[...]), U(dgs_p[:, tl]), NN) + dot(U(wu_p[...]), U(dus_p[:, tl]), NN)
        ob = [U(at[OB + b, 0:TS // 2, :]) for b in range(15)]
        o = jnp.concatenate(ob[:4], axis=1)
        dq = jnp.concatenate(ob[4:], axis=1)
        a_t = dot(U(wopt_p[...]), o, NT)
        dxa = dot(U(wp_p[...]), dq, NT) + dxf
        dwot[...] += dot(U(dat_p[:, tl]), o, NN)
        xa = U(xat_p[:, tl])
        dwp[...] += dot(xa, dq, NN)
        g = grow[:, tl]
        b_ = bt[:, tl]
        out_s[:, tl] = (g * a_t + (1.0 - g) * b_).astype(bf)
        dg = jnp.sum(dyt[:, tl].astype(f32) * (a_t - b_), axis=0, keepdims=True)
        ds = dg * g * (1.0 - g)
        gc = gwcol[...]
        dx_s[:, tl] = (dxa + jnp.concatenate([gc, gc], axis=1) * ds).astype(bf)
        t = xa.astype(f32) * ds
        dgacc[...] += t[:, 0:128] + t[:, 128:256]
        if not last:
            shuffle()

    def tile(i, carry):
        tile_body(i, False)
        for c in tcopies(i) + ocopies(i):
            c.start()
        return carry

    jax.lax.fori_loop(0, NT_ - 1, tile, 0)

    tile_body(NT_ - 1, True)
    for p in wunit_parts(NT_ + 3):
        p()

    def scatter(rows16, start):
        for b in range(3):
            perm[b, pl.ds(start, 16, stride=DH), :] = rows16[:, 128 * b:128 * (b + 1)]
        perm[3, pl.ds(start, 16, stride=DH), :] = jnp.concatenate([rows16[:, 384:448], jnp.zeros((16, 64), f32)], axis=1)

    def perm_load(rows):
        return jnp.concatenate([perm[0, 0:rows, :], perm[1, 0:rows, :], perm[2, 0:rows, :], perm[3, 0:rows, 0:64]], axis=1)

    dwpt = dwp[...].T
    for t in range(3):
        for d in range(DH):
            r = prow(t, d)
            scatter(dwpt[r:r + 16, :], D * t + d)
    dwqkv_s[...] = perm_load(3 * D).astype(bf).T
    dwo_pm = dwot[...].T
    for d in range(DH):
        scatter(dwo_pm[16 * d:16 * d + 16, :], d)
    dwo_s[...] = perm_load(D).astype(bf)
    dgw_s[...] = jnp.sum(dgacc[...].T, axis=0).astype(bf)
    fin = [cp(dwqkv_s, dwqkv_h, isem.at[6]), cp(dwo_s, dwo_h, isem.at[7]), cp(dgw_s, dgw_h, isem.at[8])]
    for c in tcopies(NT_ - 1) + ocopies(NT_ - 1) + ocopies(NT_ + 2) + ocopies(NT_ + 3) + fin:
        c.start()

    def bwd_only(j, carry):
        for p, c in zip(wunit_parts(j), ocopies(j)):
            p()
            c.start()
        return carry

    jax.lax.fori_loop(NT_ + 4, NFB, bwd_only, 0)

    for c in fin:
        c.wait()
    for i in range(NT_):
        for c in tcopies(i):
            c.wait()
    for j in range(NFB):
        for c in ocopies(j):
            c.wait()


@jax.jit
def pallas_gated_mix__sliding_local_dilated__swiglu_ffn__prompt_kernel(
    A_x, A_wqkv, A_wo, B_x, B_w_gate, B_w_up, B_w_down, gate_w, grad_out):
    del B_x
    V = pltpu.VMEM
    scratch = [
        V((D, S), bf), V((D, S), bf), V((D, 3 * D), bf), V((D, D), bf),
        V((D, F), bf), V((D, F), bf), V((D, F), bf), V((D,), bf),
        V((D // 2, S), f32), V((D // 2, S), f32), V((D // 2, S), f32),
        V((SP // 2, D), f32), V((SP // 2, D), f32),
        V((D // 2, F), f32), V((D // 2, F), f32), V((3, TFF // 2, D), f32),
        V((D // 2, NQ), f32), V((NQ // 2, D), f32), V((NO // 2, D), f32), V((D // 2, NO), f32),
        V((F // 2, S), f32), V((F // 2, S), f32), V((F // 2, S), f32),
        V((D, S), f32), V((1, S), f32), V((D, 128), f32),
        V((D, NQ), f32), V((D, NO), f32), V((D, 128), f32),
        V((NB, WS, 128), f32), V((15, TS, 128), f32), V((4, 3 * D, 128), f32),
        V((D, S), bf), V((D, S), bf), V((D, 3 * D), bf), V((D, D), bf),
        V((D, F), bf), V((D, F), bf), V((D, F), bf), V((D,), bf),
        pltpu.SMEM((1,), jnp.int32),
        pltpu.SemaphoreType.DMA((10 + 3 * NFF,)),
        pltpu.SemaphoreType.DMA((2, NT_)), pltpu.SemaphoreType.DMA((3, NFB)),
    ]
    sd = jax.ShapeDtypeStruct
    out_shape = [sd((D, S), bf), sd((D, S), bf), sd((D, 3 * D), bf), sd((D, D), bf),
                 sd((D, F), bf), sd((D, F), bf), sd((D, F), bf), sd((D,), bf)]
    anyspec = pl.BlockSpec(memory_space=pl.ANY)
    outt, dxt, dwqkv, dwo, dwg, dwu, dwdt, dgw = pl.pallas_call(
        kernel,
        in_specs=[anyspec] * 8,
        out_specs=[anyspec] * 8,
        out_shape=out_shape,
        scratch_shapes=scratch,
        compiler_params=pltpu.CompilerParams(
            vmem_limit_bytes=120 * 1024 * 1024,
            disable_semaphore_checks=True),
        name="gated_mix",
    )(A_x[0].T, A_wqkv, A_wo, B_w_gate, B_w_up, B_w_down.T, gate_w, grad_out[0].T)
    return outt.T[None], dxt.T[None], dwqkv, dwo, dwg, dwu, dwdt.T, dgw
```
